```python
import os as _os
_os.environ.setdefault("JAX_PLATFORMS", "cpu")
import jax
import jax.numpy as jnp

def _softmax(x, axis=-1):
    return jax.nn.softmax(x, axis=axis)
def _gelu(x):
    return jax.nn.gelu(x, approximate=True)
def _silu(x):
    return jax.nn.silu(x)
def _sigmoid(x):
    return jax.nn.sigmoid(x)
def _layernorm(x, axis=-1, eps=1e-5):
    m = jnp.mean(x, axis=axis, keepdims=True)
    v = jnp.var(x, axis=axis, keepdims=True)
    return (x - m) / jnp.sqrt(v + eps)
def _scatter_add(tgt, idx, src, axis=0):
    return tgt.at[idx].add(src)
def _segment_sum(src, seg, n):
    return jax.ops.segment_sum(src, seg, n)
class _Rng:
    def __init__(self, key):
        self._k = key
    def _next(self):
        self._k, sub = jax.random.split(self._k)
        return sub
    def normal(self, shape):
        return jax.random.normal(self._next(), shape, dtype=jnp.bfloat16)
    def randint(self, lo, hi, shape):
        return jax.random.randint(self._next(), shape, lo, hi, dtype=jnp.int32)
    def uniform(self, shape, lo=0.0, hi=1.0):
        return jax.random.uniform(self._next(), shape, jnp.bfloat16, lo, hi)
    def permutation(self, n):
        return jax.random.permutation(self._next(), n)


kernel_name = 'parallel_sum__ssm_conv_h3__dense_activation_silu__prompt'

def setup_inputs():
    _rng = _Rng(jax.random.key(int.from_bytes(__import__("os").urandom(4), "little")))
    _w = (lambda a: (lambda t: t.astype(jnp.bfloat16) if jnp.issubdtype(t.dtype, jnp.floating) else t)(jnp.asarray(a)))
    def _A_setup():
        B, S, D = 1, 2048, 448
        ks = 4
        return {
            "q": _w((lambda *s: _rng.normal(s) * 0.05)(B, S, D)),
            "k": _w((lambda *s: _rng.normal(s) * 0.2)(B, S, D)),
            "v": _w((lambda *s: _rng.normal(s) * 0.2)(B, S, D)),
            "shift_k": _w((lambda *s: _rng.normal(s) * 0.2)(D, ks) * 0.5),
            "ssm_k": _w((lambda *s: _rng.normal(s) * 0.2)(D, S) * (1.0 / S ** 0.5)),
            "ssm_D": _w((lambda *s: _rng.normal(s) * 0.2)(D)),
        }
    _A_in = _A_setup()

    def _B_setup():
        B, S, D, F = 1, 2048, 448, 1792
        return {
            "x": _w((lambda *s: _rng.normal(s) * 0.05)(B, S, D)),
            "w1": _w((lambda *s: _rng.normal(s) * 0.05)(D, F) * (D ** -0.5)),
            "w2": _w((lambda *s: _rng.normal(s) * 0.05)(F, D) * (F ** -0.5)),
        }
    _B_in = _B_setup()

    return {
        "A_q": _A_in["q"],
        "A_k": _A_in["k"],
        "A_v": _A_in["v"],
        "A_shift_k": _A_in["shift_k"],
        "A_ssm_k": _A_in["ssm_k"],
        "A_ssm_D": _A_in["ssm_D"],
        "B_x": _B_in["x"],
        "B_w1": _B_in["w1"],
        "B_w2": _B_in["w2"],
    }

def reference(A_q, A_k, A_v, A_shift_k, A_ssm_k, A_ssm_D, B_x, B_w1, B_w2):
    def _A_ref(q, k, v, shift_k, ssm_k, ssm_D):
        B, S, D = q.shape
        ks = shift_k.shape[-1]
        k_pad = jnp.pad(k, ((0, 0), (ks - 1, 0), (0, 0)))
        k_shift = jnp.zeros_like(k)
        for t in range(ks):
            k_shift = k_shift + k_pad[:, t:t + S, :] * shift_k[:, ks - 1 - t][None, None, :]
        kv = k_shift * v
        L = 2 * S
        kv_pad = jnp.pad(kv, ((0, 0), (0, S), (0, 0)))
        kf_pad = jnp.pad(ssm_k, ((0, 0), (0, S)))
        kv_f = (lambda x, axes=(-2,-1): jnp.fft.rfft2(x.astype(jnp.float32), axes=axes))(kv_pad[:, None, :, :], axes=(1, 2))
        kf_f = (lambda x, axes=(-2,-1): jnp.fft.rfft2(x.astype(jnp.float32), axes=axes))(kf_pad[:, None, :], axes=(1, 2))
        kf_f = (lambda x, *d: x.transpose(*d))(kf_f, 1, 2, 0)
        y_f = kv_f * kf_f[None, :, :, :]
        y = (lambda x, s, axes=(-2,-1): jnp.fft.irfft2(x, s=s, axes=axes).astype(jnp.bfloat16))(y_f, (1, L), axes=(1, 2))[:, 0, :S, :]
        y = y + kv * ssm_D[None, None, :]
        return q * y

    def _B_ref(x, w1, w2):
        h = jnp.einsum("bsd,df->bsf", x, w1)
        h = _silu(h)
        out = jnp.einsum("bsf,fd->bsd", h, w2)
        return out

    x = A_q
    xn = _layernorm(x, axis=-1)
    return x + _A_ref(xn, A_k, A_v, A_shift_k, A_ssm_k, A_ssm_D) + _B_ref(xn, B_w1, B_w2)
```

```python
import functools
import numpy as np, jax, jax.numpy as jnp
from jax import lax
from jax.experimental import pallas as pl
from jax.experimental.pallas import tpu as pltpu
import ml_dtypes

S, D, F = 2048, 448, 1792
C = 128; NC = S // C
bf = jnp.bfloat16; f32 = jnp.float32; i32 = jnp.int32

def _tables():
    t = np.arange(512, dtype=np.float64)[:, None]; k = np.arange(128, dtype=np.float64)[None, :]
    th = 2 * np.pi * (k + 0.5) * t / 256.0
    wf = np.concatenate([np.cos(th), -np.sin(th)], axis=1)
    wi = (wf.T / 64.0)
    def pack(a):
        b = a.astype(np.float32).astype(ml_dtypes.bfloat16).view(np.uint16).astype(np.uint32)
        return (b[0::2] | (b[1::2] << 16)).astype(np.uint32).view(np.int32)
    return pack(wf), pack(wi)
WF_P, WI_P = _tables()
LP = {'XLA_TPU_FORCE_LP_LLO_SCHEDULER': True}

def make(BT=256, RS=8, vmem=110 << 20, flags=LP, W1P=(7, 7), waitsfirst=False, NCH=1, gate=1, tailsplit=False,
         UQ=None, MQ=None, FQ=None, RU=112, ugate='k', cform=True, trig=True, lngate=False, chainadd=True, w2t=0, PLAN=0, P0=(6, 1, 7), lnR2=True, lnseq=True, lnre=0, R2='a', lnforce=False, whole=1, DQ=None, w0split=True, LNQ=None):
    NB = S // BT; CPB = BT // C
    assert sum(W1P) == 14
    W1O = [sum(W1P[:j]) for j in range(len(W1P))]
    NP1 = len(W1P)
    def kern(x_h, k_h, v_h, sk_h, f_h, d_h, w1_h, w2_h, wf_h, wi_h, o_h,
             x_v, k_v, v_v, f_v, sk_v, d_v, w1_v, w2_v, wf_v, wi_v, o_v, sems, osem):
        cnt = [0]; allc = []
        def dma(src, dst):
            c = pltpu.make_async_copy(src, dst, sems.at[cnt[0]]); cnt[0] += 1
            allc.append(c); return c
        sl = lambda i, n=1: pl.ds(i * BT, n * BT)
        cs = lambda s, n=1: pl.ds(s * C, n * C)
        c_sk = dma(sk_h, sk_v); c_d = dma(d_h, d_v)
        c_x0 = dma(x_h.at[:, sl(0)], x_v.at[:, sl(0)])
        c_w1 = [dma(w1_h.at[:, pl.ds(W1O[j] * 128, W1P[j] * 128)], w1_v.at[:, pl.ds(W1O[j] * 128, W1P[j] * 128)]) for j in range(NP1)]
        c_x1 = dma(x_h.at[:, sl(1)], x_v.at[:, sl(1)])
        c_w2 = dma(w2_h, w2_v)
        c_wf = dma(wf_h, wf_v)
        c_x23 = dma(x_h.at[:, sl(2, 6)], x_v.at[:, sl(2, 6)])
        c_f0 = dma(f_h.at[:, cs(0, 8)], f_v.at[:, cs(0, 8)])
        c_k0 = dma(k_h.at[:, cs(0, 8)], k_v.at[:, cs(0, 8)])
        c_v0 = dma(v_h.at[:, cs(0, 8)], v_v.at[:, cs(0, 8)])
        c_f1 = dma(f_h.at[:, cs(8, 8)], f_v.at[:, cs(8, 8)])
        c_wi = dma(wi_h, wi_v)
        c_k1 = dma(k_h.at[:, cs(8, 8)], k_v.at[:, cs(8, 8)])
        c_v1 = dma(v_h.at[:, cs(8, 8)], v_v.at[:, cs(8, 8)])
        for c in allc: c.start()
        waited = set()
        def W(*cs_):
            for c in cs_:
                if id(c) not in waited:
                    waited.add(id(c)); c.wait()
        if waitsfirst: W(*allc)

        st = {}
        def params():
            skf = sk_v[...].astype(f32)
            st['skb'] = [jnp.broadcast_to(skf[j:j + 1, :], (128, D)).T for j in range(4)]
            st['db'] = jnp.broadcast_to(d_v[...].astype(f32).reshape(1, D), (128, D)).T
            st['lane'] = lax.broadcasted_iota(i32, (D, C), 1)
        def w1prep(j):
            st['w1t', j] = w1_v[:, pl.ds(W1O[j] * 128, W1P[j] * 128)].T
        def ln(i, gate=None):
            if lnre and i >= 2:
                z = st['zz']
                ld = lambda q: x_v[:, pl.ds(pl.multiple_of(z[q] + i * BT, C), BT)].astype(f32)
                x1 = ld(0)
                if gate is not None: x1 = jnp.where(st['neverX'], gate, x1)
                m = jnp.mean(x1, axis=0, keepdims=True)
                xc = ld(1) - m
                var = jnp.mean(xc * xc, axis=0, keepdims=True)
                r = 0.5 * lax.rsqrt(var + 1e-5)
                xn = (ld(2) - m) * r
            else:
                x = x_v[:, sl(i)].astype(f32)
                if gate is not None: x = jnp.where(st['neverX'], gate, x)
                m = jnp.mean(x, axis=0, keepdims=True)
                xc = x - m
                var = jnp.mean(xc * xc, axis=0, keepdims=True)
                xn = xc * (0.5 * lax.rsqrt(var + 1e-5))
            st['xn', i] = xn
            st['xh', i] = xn.astype(bf)
        def pieces(i): return [(sum(P0[:j]), P0[j]) for j in range(len(P0))] if i < whole else [(0, 14)]
        def w1rows(o, n):
            parts = []
            for q in range(NP1):
                lo = max(o, W1O[q]); hi = min(o + n, W1O[q] + W1P[q])
                if lo < hi: parts.append(st['w1t', q][(lo - W1O[q]) * 128:(hi - W1O[q]) * 128])
            return parts[0] if len(parts) == 1 else jnp.concatenate(parts, axis=0)
        def f1(i, j):
            o, n = pieces(i)[j]
            w = w1rows(o, n)
            h = jnp.dot(w, st['xh', i], preferred_element_type=f32)
            a = (h + h * jnp.tanh(h)).astype(bf)
            if lnforce and i >= 3 and ('xh', i + 1) in st and j == len(pieces(i)) - 1:
                a = jnp.concatenate([a[:-D], pltpu.bitcast(jnp.where(jnp.tile(wf_v[0:8, 0:C], (D // 16, BT // C)) == 0x7F7F7F7F, pltpu.bitcast(st['xh', i + 1], i32), pltpu.bitcast(a[-D:], i32)), bf)], axis=0)
            st['a', i, j] = a
        def f2(i, j=0, n=None):
            a = st['a', i, 0] if len(pieces(i)) == 1 else jnp.concatenate([st['a', i, q] for q in range(len(pieces(i)))], axis=0)
            if w2t and i >= w2t: w = pltpu.bitcast(st['w2p'], bf)
            else: w = w2_v[...]
            if n is None:
                st['b', i] = jnp.dot(w, a, preferred_element_type=f32)
            else:
                st['bn', i, n] = jnp.dot(w, a[:, n * C:(n + 1) * C], preferred_element_type=f32)
        def w2prep():
            st['w2p'] = pltpu.bitcast(w2_v[...], i32)
        def bval(t1):
            i, c = divmod(t1, CPB)
            if ('bn', i, c) in st: return st['bn', i, c]
            return st['b', i][:, c * C:(c + 1) * C]
        def ucalc(s, trig=None):
            us = []
            for r0 in range(0, D, RU):
                rs = slice(r0, r0 + RU)
                k = k_v[rs, cs(s)].astype(f32)
                kp = k_v[rs, cs(s - 1)].astype(f32) if s > 0 else None
                w0, w1, w2, w3 = (w[rs] for w in st['skb'])
                if 'chain' in st:
                    k = jnp.where(st['neverD'][0:RU], jnp.tile(st['chain'], (RU // 8, 1)), k)
                def shift(j):
                    m = jnp.where(st['lane'][0:RU] >= C - j, 0.0 if kp is None else kp, k)
                    return pltpu.roll(m, j, 1)
                u = (k * w0 + shift(1) * w1 + shift(2) * w2 + shift(3) * w3) * v_v[rs, cs(s)].astype(f32)
                st['chain'] = u[RU - 8:]
                us.append(u.astype(bf))
            st['u', s] = jnp.concatenate(us, axis=0)
        def wf_t(s): return pltpu.bitcast(wf_v[pl.ds((s % 4) * 64, 64), :], bf)
        def dftu(s):
            r = jnp.dot(st.pop(('u', s)), wf_t(s), preferred_element_type=f32)
            st['U', s] = (r[:, :C], r[:, C:])
        def dftf(s):
            r = jnp.dot(f_v[:, cs(s)], wf_t(s), preferred_element_type=f32)
            if s == 0: r = r + jnp.concatenate([st['db'], jnp.zeros((D, C), f32)], axis=1)
            st['Fq', s] = r
            g = r if (s == 0 or cform) else r + st['Fq', s - 1]
            st['G', s] = (g[:, :C], g[:, C:])
        def mac(t1, r0):
            rs = slice(r0, r0 + RS)
            ch = (r0 // RS) % NCH
            for s1 in range(t1 + 1):
                dl = t1 - s1
                gr = st['G', dl][0][rs]; gi = st['G', dl][1][rs]; ur = st['U', s1][0][rs]; ui = st['U', s1][1][rs]
                if s1 == 0:
                    are = gr * ur - gi * ui; aim = gr * ui + gi * ur
                    if 'chain' in st:
                        are = jnp.where(st['never'], st['chain'], are); aim = jnp.where(st['never'], st['chain'], aim)
                else:
                    are = are + gr * ur; are = are - gi * ui
                    aim = aim + gr * ui; aim = aim + gi * ur
            st['chain'] = (are + aim) if chainadd else aim
            y = jnp.concatenate([are, aim], axis=1)
            if cform:
                st['Cq', t1, r0] = y
                if t1 > 0: y = y + st.pop(('Cq', t1 - 1, r0))
            st.setdefault(('Y', t1), []).append(y)
        def idft(t1):
            wi = pltpu.bitcast(wi_v[:, pl.ds((t1 % 4) * C, C)], bf)
            Y = jnp.concatenate(st.pop(('Y', t1)), axis=0).astype(bf)
            y = jnp.dot(Y, wi, preferred_element_type=f32)
            i, c = divmod(t1, CPB)
            y2 = y
            st['z', t1] = x_v[:, cs(t1)].astype(f32) + st['xn', i][:, c * C:(c + 1) * C] * y2
        def final(t1):
            o_v[:, cs(t1)] = (st.pop(('z', t1)) + bval(t1)).astype(bf)
        ostarted = []
        def ostart(c0, n):
            c = pltpu.make_async_copy(o_v.at[:, cs(c0, n)], o_h.at[:, cs(c0, n)], osem.at[len(ostarted)])
            c.start(); ostarted.append(c)
        P = functools.partial
        def macs(t1): return [P(mac, t1, r0) for r0 in range(0, D, RS)]
        def interleave(main, side):
            out = []; n = len(main); m = len(side); j = 0
            for q, t in enumerate(main):
                out.append(t)
                tgt = (q + 1) * m // n
                while j < tgt: out.append(side[j]); j += 1
            assert j == m
            return out
        def run(l):
            for t in l: t()
        def ffn(i):
            return [P(f1, i, 0), P(f2, i)]
        lnq = {}
        W(c_sk, c_d, c_x0); params(); ln(0); W(c_w1[0]); w1prep(0); f1(0, 0)
        W(c_w1[1], c_x1); w1prep(1); ln(1)
        for j in range(1, len(P0)): f1(0, j)
        f1(1, 0)
        W(c_w2, c_wf, c_x23)
        st['never'] = wf_v[0:RS, 0:C] == 0x7F7F7F7F
        st['neverD'] = jnp.tile(wf_v[0:8, 0:C], (RU // 8, 1)) == 0x7F7F7F7F
        st['neverX'] = jnp.tile(wf_v[0:8, 0:C], (D // 8, BT // C)) == 0x7F7F7F7F
        z0 = jnp.max(jnp.where(st['never'], 1, 0))
        st['zz'] = [z0, z0 * z0, z0 * z0 * z0 + z0]
        if R2 == 'a':
            ln(2); f2(0); ln(3, st['xn', 2]); ln(4, st['xn', 3])
            f2(1); ln(5, st['xn', 4]); ln(6, st['xn', 5]); ln(7, st['xn', 6])
        elif R2 == 'b':
            ln(2); f2(0); ln(3, st['b', 0]); ln(4, st['xn', 3])
            f2(1); ln(5, st['xn', 4])
            lnq.update({'W2': [6], 'W3': [7]})
        elif R2 == 'c':
            ln(2); f2(0); ln(3, st['xn', 2]); ln(4, st['xn', 3])
            f2(1); ln(5, st['b', 0]); ln(6, st['xn', 5]); ln(7, st['xn', 6])
        if w2t: w2prep()
        W(c_f0, c_k0, c_v0)
        def U(*ss):
            l = []
            for s_ in ss: l += [P(ucalc, s_), P(dftu, s_), P(dftf, s_)]
            return l
        def M(*ts):
            l = []
            for t1 in ts: l += macs(t1)
            return l
        def FI(*bs):
            l = []
            for b in bs: l += [P(idft, b * CPB + c) for c in range(CPB)] + [P(final, b * CPB + c) for c in range(CPB)] + [P(ostart, b * CPB, CPB)]
            return l
        plans = {
          0: {2: (U(0, 1, 2, 3, 4, 5), M(0, 1, 2, 3)),
              3: (U(6) + M(4) + U(7) + M(5), FI(0, 1) + U(8) + M(6) + U(9) + M(7)),
              4: (U(10, 11) + M(8), FI(2, 3) + M(9, 10)),
              5: (U(12, 13) + M(11), FI(4) + M(12)),
              6: (U(14, 15) + M(13), FI(5) + M(14)),
              7: (M(15), FI(6))},
          1: {2: (U(0, 1, 2, 3, 4, 5), M(0, 1, 2, 3)),
              3: (U(6) + M(4) + U(7) + M(5), U(8) + M(6) + FI(0) + U(9) + M(7)),
              4: (U(10, 11) + M(8) + FI(1), M(9, 10) + FI(2)),
              5: (U(12, 13) + M(11) + FI(3), M(12) + FI(4)),
              6: (U(14, 15) + M(13), FI(5) + M(14)),
              7: (M(15), FI(6))},
        }[PLAN]
        for i in range(2, NB):
            if i == 3: W(*allc)
            for b in lnq.get({2: 'W2', 3: 'W3'}.get(i, i), []): ln(b)
            A, B = plans[i]
            main = ffn(i)
            assert len(main) == 2
            main[0](); run(A)
            if i == NB - 1 and tailsplit:
                run(B); idft(14); idft(15)
            else:
                main[1](); run(B)
        if tailsplit:
            f2(NB - 1, 0, 0); final(14); ostart(14, 1)
            f2(NB - 1, 0, 1); final(15); ostart(15, 1)
        else:
            for c in range(CPB): idft(14 + c)
            for c in range(CPB): final(14 + c)
            ostart(14, 2)
        for c in ostarted: c.wait()

    def f(A_q, A_k, A_v, A_shift_k, A_ssm_k, A_ssm_D, B_x, B_w1, B_w2):
        any_ = pl.BlockSpec(memory_space=pl.ANY)
        V = pltpu.VMEM
        o = pl.pallas_call(kern,
            in_specs=[any_] * 10, out_specs=any_,
            out_shape=jax.ShapeDtypeStruct((D, S), bf),
            scratch_shapes=[V((D, S), bf), V((D, S), bf), V((D, S), bf), V((D, S), bf), V((4, D), bf), V((D,), bf), V((D, F), bf), V((D, F), bf),
                            V((256, 256), i32), V((128, 512), i32), V((D, S), bf),
                            pltpu.SemaphoreType.DMA((24,)), pltpu.SemaphoreType.DMA((16,))],
            compiler_params=pltpu.CompilerParams(vmem_limit_bytes=vmem, **({'flags': flags} if flags else {})),
        )(A_q.reshape(S, D).T, A_k.reshape(S, D).T, A_v.reshape(S, D).T, A_shift_k.T, A_ssm_k, A_ssm_D, B_w1, B_w2.T,
          jnp.asarray(WF_P), jnp.asarray(WI_P))
        return o.T.reshape(1, S, D)
    return f


_kernel_impl = make(R2='b')


@jax.jit
def pallas_parallel_sum__ssm_conv_h3__dense_activation_silu__prompt_kernel(
        A_q, A_k, A_v, A_shift_k, A_ssm_k, A_ssm_D, B_x, B_w1, B_w2):
    return _kernel_impl(A_q, A_k, A_v, A_shift_k, A_ssm_k, A_ssm_D, B_x, B_w1, B_w2)
```

```python
import functools

import jax
import jax.numpy as jnp
import ml_dtypes
import numpy as np
from jax import lax
from jax.experimental import pallas as pl
from jax.experimental.pallas import tpu as pltpu

S, D, F = 2048, 448, 1792
C = 128
NC = S // C
BT = 256
NB = S // BT
CPB = BT // C
RS = 8
RU = 112
W1P = (7, 7)
P0 = (6, 1, 7)
MAGIC = 0x7F7F7F7F
bf, f32, i32 = jnp.bfloat16, jnp.float32, jnp.int32


def _tables():
    t = np.arange(512, dtype=np.float64)[:, None]
    k = np.arange(128, dtype=np.float64)[None, :]
    th = 2 * np.pi * (k + 0.5) * t / 256.0
    wf = np.concatenate([np.cos(th), -np.sin(th)], axis=1)
    wi = wf.T / 64.0

    def pack(a):
        b = a.astype(np.float32).astype(ml_dtypes.bfloat16).view(np.uint16).astype(np.uint32)
        return (b[0::2] | (b[1::2] << 16)).astype(np.uint32).view(np.int32)

    return pack(wf), pack(wi)


WF_P, WI_P = _tables()
W1O = [sum(W1P[:j]) for j in range(len(W1P))]


def _kernel(x_h, k_h, v_h, sk_h, f_h, d_h, w1_h, w2_h, wf_h, wi_h, o_h,
            x_v, k_v, v_v, f_v, sk_v, d_v, w1_v, w2_v, wf_v, wi_v, o_v, sems, osem):
    allc = []

    def dma(src, dst):
        c = pltpu.make_async_copy(src, dst, sems.at[len(allc)])
        allc.append(c)
        return c

    sl = lambda i, n=1: pl.ds(i * BT, n * BT)
    cs = lambda s, n=1: pl.ds(s * C, n * C)
    c_sk = dma(sk_h, sk_v)
    c_d = dma(d_h, d_v)
    c_x0 = dma(x_h.at[:, sl(0)], x_v.at[:, sl(0)])
    c_w1 = [dma(w1_h.at[:, pl.ds(W1O[j] * 128, W1P[j] * 128)], w1_v.at[:, pl.ds(W1O[j] * 128, W1P[j] * 128)])
            for j in range(len(W1P))]
    c_x1 = dma(x_h.at[:, sl(1)], x_v.at[:, sl(1)])
    c_w2 = dma(w2_h, w2_v)
    c_wf = dma(wf_h, wf_v)
    c_x23 = dma(x_h.at[:, sl(2, 2)], x_v.at[:, sl(2, 2)])
    c_x4 = dma(x_h.at[:, sl(4)], x_v.at[:, sl(4)])
    c_f0 = dma(f_h.at[:, cs(0, 8)], f_v.at[:, cs(0, 8)])
    c_k0 = dma(k_h.at[:, cs(0, 8)], k_v.at[:, cs(0, 8)])
    c_v0 = dma(v_h.at[:, cs(0, 8)], v_v.at[:, cs(0, 8)])
    dma(f_h.at[:, cs(8, 8)], f_v.at[:, cs(8, 8)])
    dma(wi_h, wi_v)
    dma(x_h.at[:, sl(5, 3)], x_v.at[:, sl(5, 3)])
    dma(k_h.at[:, cs(8, 8)], k_v.at[:, cs(8, 8)])
    dma(v_h.at[:, cs(8, 8)], v_v.at[:, cs(8, 8)])
    for c in allc:
        c.start()
    waited = []

    def wait(*copies):
        for c in copies:
            if not any(c is w for w in waited):
                waited.append(c)
                c.wait()

    st = {}

    def params():
        skf = sk_v[...].astype(f32)
        st['skb'] = [jnp.broadcast_to(skf[j:j + 1, :], (128, D)).T for j in range(4)]
        st['db'] = jnp.broadcast_to(d_v[...].astype(f32).reshape(1, D), (128, D)).T
        st['lane'] = lax.broadcasted_iota(i32, (D, C), 1)

    def w1prep(j):
        st['w1t', j] = w1_v[:, pl.ds(W1O[j] * 128, W1P[j] * 128)].T

    def ln(i, gate=None, chain=False):
        if chain and 'chain' in st:
            gate = jnp.tile(st['chain'], (D // 8, BT // C))
        x = x_v[:, sl(i)].astype(f32)
        if gate is not None:
            x = jnp.where(st['neverX'], gate, x)
        m = jnp.mean(x, axis=0, keepdims=True)
        xc = x - m
        var = jnp.mean(xc * xc, axis=0, keepdims=True)
        r = 0.5 * lax.rsqrt(var + 1e-5)
        xn = xc * r
        st['mr', i] = (m, r)
        if chain:
            st['chain'] = xn[D - 8:, BT - C:]
        st['xh', i] = xn.astype(bf)

    def pieces(i):
        return [(sum(P0[:j]), P0[j]) for j in range(len(P0))] if i == 0 else [(0, 14)]

    def w1rows(o, n):
        parts = []
        for q in range(len(W1P)):
            lo, hi = max(o, W1O[q]), min(o + n, W1O[q] + W1P[q])
            if lo < hi:
                parts.append(st['w1t', q][(lo - W1O[q]) * 128:(hi - W1O[q]) * 128])
        return parts[0] if len(parts) == 1 else jnp.concatenate(parts, axis=0)

    def f1(i, j):
        o, n = pieces(i)[j]
        h = jnp.dot(w1rows(o, n), st['xh', i], preferred_element_type=f32)
        st['a', i, j] = (h + h * jnp.tanh(h)).astype(bf)

    def f2(i, n=None):
        np_ = len(pieces(i))
        a = st['a', i, 0] if np_ == 1 else jnp.concatenate([st['a', i, q] for q in range(np_)], axis=0)
        if n is None:
            st['b', i] = jnp.dot(w2_v[...], a, preferred_element_type=f32)
        else:
            st['bn', i, n] = jnp.dot(w2_v[...], a[:, n * C:(n + 1) * C], preferred_element_type=f32)

    def bval(t1):
        i, c = divmod(t1, CPB)
        if ('bn', i, c) in st:
            return st['bn', i, c]
        return st['b', i][:, c * C:(c + 1) * C]

    def ucalc(s):
        us = []
        for r0 in range(0, D, RU):
            rs = slice(r0, r0 + RU)
            k = k_v[rs, cs(s)].astype(f32)
            kp = k_v[rs, cs(s - 1)].astype(f32) if s > 0 else None
            w0, w1, w2, w3 = (w[rs] for w in st['skb'])
            if 'chain' in st:
                k = jnp.where(st['neverD'][0:RU], jnp.tile(st['chain'], (RU // 8, 1)), k)

            def shift(j):
                m = jnp.where(st['lane'][0:RU] >= C - j, 0.0 if kp is None else kp, k)
                return pltpu.roll(m, j, 1)

            u = (k * w0 + shift(1) * w1 + shift(2) * w2 + shift(3) * w3) * v_v[rs, cs(s)].astype(f32)
            st['chain'] = u[RU - 8:]
            us.append(u.astype(bf))
        st['u', s] = jnp.concatenate(us, axis=0)

    def wf_t(s):
        return pltpu.bitcast(wf_v[pl.ds((s % 4) * 64, 64), :], bf)

    def dftu(s):
        r = jnp.dot(st.pop(('u', s)), wf_t(s), preferred_element_type=f32)
        st['U', s] = (r[:, :C], r[:, C:])

    def dftf(s):
        r = jnp.dot(f_v[:, cs(s)], wf_t(s), preferred_element_type=f32)
        if s == 0:
            r = r + jnp.concatenate([st['db'], jnp.zeros((D, C), f32)], axis=1)
        st['G', s] = (r[:, :C], r[:, C:])

    def mac(t1, r0):
        rs = slice(r0, r0 + RS)
        for s1 in range(t1 + 1):
            dl = t1 - s1
            gr, gi = st['G', dl][0][rs], st['G', dl][1][rs]
            ur, ui = st['U', s1][0][rs], st['U', s1][1][rs]
            if s1 == 0:
                are = gr * ur - gi * ui
                aim = gr * ui + gi * ur
                if 'chain' in st:
                    are = jnp.where(st['never'], st['chain'], are)
                    aim = jnp.where(st['never'], st['chain'], aim)
            else:
                are = are + gr * ur
                are = are - gi * ui
                aim = aim + gr * ui
                aim = aim + gi * ur
        st['chain'] = are + aim
        y = jnp.concatenate([are, aim], axis=1)
        st['Cq', t1, r0] = y
        if t1 > 0:
            y = y + st.pop(('Cq', t1 - 1, r0))
        st.setdefault(('Y', t1), []).append(y)

    def idft(t1):
        wi = pltpu.bitcast(wi_v[:, pl.ds((t1 % 4) * C, C)], bf)
        Y = jnp.concatenate(st.pop(('Y', t1)), axis=0).astype(bf)
        y2 = jnp.dot(Y, wi, preferred_element_type=f32)
        i, c = divmod(t1, CPB)
        xx = x_v[:, cs(t1)].astype(f32)
        m, r = st['mr', i]
        xn = (xx - m[:, c * C:(c + 1) * C]) * r[:, c * C:(c + 1) * C]
        st['z', t1] = xx + xn * y2

    def final(t1):
        o_v[:, cs(t1)] = (st.pop(('z', t1)) + bval(t1)).astype(bf)

    ostarted = []

    def ostart(c0, n):
        c = pltpu.make_async_copy(o_v.at[:, cs(c0, n)], o_h.at[:, cs(c0, n)], osem.at[len(ostarted)])
        c.start()
        ostarted.append(c)

    P = functools.partial

    def U(*ss):
        return [t for s in ss for t in (P(ucalc, s), P(dftu, s), P(dftf, s))]

    def M(*ts):
        return [P(mac, t1, r0) for t1 in ts for r0 in range(0, D, RS)]

    def FI(*bs):
        l = []
        for b in bs:
            l += [P(idft, b * CPB + c) for c in range(CPB)]
            l += [P(final, b * CPB + c) for c in range(CPB)]
            l += [P(ostart, b * CPB, CPB)]
        return l

    def run(l):
        for t in l:
            t()

    wait(c_x0)
    ln(0)
    wait(c_w1[0])
    w1prep(0)
    f1(0, 0)
    wait(c_w1[1], c_x1)
    w1prep(1)
    ln(1)
    for j in range(1, len(P0)):
        f1(0, j)
    f1(1, 0)
    wait(c_w2, c_wf, c_x23, c_sk, c_d)
    params()
    st['never'] = wf_v[0:RS, 0:C] == MAGIC
    st['neverD'] = jnp.tile(wf_v[0:8, 0:C], (RU // 8, 1)) == MAGIC
    st['neverX'] = jnp.tile(wf_v[0:8, 0:C], (D // 8, BT // C)) == MAGIC
    ln(2)
    f2(0)
    ln(3, st['b', 0])
    f2(1)
    wait(c_f0, c_k0, c_v0, c_x4)
    plan = {2: (U(0, 1, 2, 3, 4, 5), M(0, 1, 2, 3)),
            3: (U(6) + M(4) + U(7) + M(5), FI(0, 1) + U(8) + M(6) + U(9) + M(7)),
            4: (U(10, 11) + M(8), FI(2, 3) + M(9, 10)),
            5: (U(12, 13) + M(11), FI(4) + M(12)),
            6: (U(14, 15) + M(13), FI(5) + M(14)),
            7: (M(15), FI(6))}
    for i in range(2, NB):
        if i == 3:
            wait(*allc)
        side_a, side_b = plan[i]
        f1(i, 0)
        if i + 2 < NB:
            ln(i + 2, None, True)
        run(side_a)
        if i < NB - 1:
            f2(i)
            run(side_b)
        else:
            run(side_b)
            idft(NC - 2)
            idft(NC - 1)
    f2(NB - 1, 0)
    final(NC - 2)
    ostart(NC - 2, 1)
    f2(NB - 1, 1)
    final(NC - 1)
    ostart(NC - 1, 1)
    for c in ostarted:
        c.wait()


@jax.jit
def pallas_parallel_sum__ssm_conv_h3__dense_activation_silu__prompt_kernel(
        A_q, A_k, A_v, A_shift_k, A_ssm_k, A_ssm_D, B_x, B_w1, B_w2):
    del B_x
    any_ = pl.BlockSpec(memory_space=pl.ANY)
    V = pltpu.VMEM
    out = pl.pallas_call(
        _kernel,
        in_specs=[any_] * 10,
        out_specs=any_,
        out_shape=jax.ShapeDtypeStruct((D, S), bf),
        scratch_shapes=[V((D, S), bf), V((D, S), bf), V((D, S), bf), V((D, S), bf), V((4, D), bf), V((D,), bf),
                        V((D, F), bf), V((D, F), bf), V((256, 256), i32), V((128, 512), i32), V((D, S), bf),
                        pltpu.SemaphoreType.DMA((24,)), pltpu.SemaphoreType.DMA((16,))],
        compiler_params=pltpu.CompilerParams(
            vmem_limit_bytes=110 << 20, flags={'XLA_TPU_FORCE_LP_LLO_SCHEDULER': True}),
    )(A_q.reshape(S, D).T, A_k.reshape(S, D).T, A_v.reshape(S, D).T, A_shift_k.T, A_ssm_k, A_ssm_D,
      B_w1, B_w2.T, jnp.asarray(WF_P), jnp.asarray(WI_P))
    return out.T.reshape(1, S, D)
```
